```python
import jax
import jax.numpy as jnp

def _softmax(x, axis=-1):
    return jax.nn.softmax(x, axis=axis)

def _gelu(x):
    return jax.nn.gelu(x, approximate=True)

def _silu(x):
    return jax.nn.silu(x)

def _sigmoid(x):
    return jax.nn.sigmoid(x)

def _layernorm(x, axis=-1, eps=1e-05):
    m = jnp.mean(x, axis=axis, keepdims=True)
    v = jnp.var(x, axis=axis, keepdims=True)
    return (x - m) / jnp.sqrt(v + eps)

def _scatter_add(tgt, idx, src, axis=0):
    return tgt.at[idx].add(src)

def _segment_sum(src, seg, n):
    return jax.ops.segment_sum(src, seg, n)

class _Rng:

    def __init__(self, key):
        self._k = key

    def _next(self):
        self._k, sub = jax.random.split(self._k)
        return sub

    def normal(self, shape):
        return jax.random.normal(self._next(), shape, dtype=jnp.bfloat16)

    def randint(self, lo, hi, shape):
        return jax.random.randint(self._next(), shape, lo, hi, dtype=jnp.int32)

    def uniform(self, shape, lo=0.0, hi=1.0):
        return jax.random.uniform(self._next(), shape, jnp.bfloat16, lo, hi)

    def permutation(self, n):
        return jax.random.permutation(self._next(), n)
kernel_name = 'adaLN_cond__sliding_local_dilated__mixer_s_mlp__prompt'

def setup_inputs():
    _rng = _Rng(jax.random.key(int.from_bytes(__import__("os").urandom(4), "little")))
    _w = lambda a: (lambda t: t.astype(jnp.bfloat16) if jnp.issubdtype(t.dtype, jnp.floating) else t)(jnp.asarray(a))

    def _A_setup():
        B, S, D = (1, 2048, 1024)
        return {'x': _w((lambda *s: _rng.normal(s) * 0.05)(B, S, D)), 'wqkv': _w((lambda *s: _rng.normal(s) * 0.05)(D, 3 * D)), 'wo': _w((lambda *s: _rng.normal(s) * 0.05)(D, D))}
    _A_in = _A_setup()

    def _B_setup():
        B, S, D, F = (1, 2048, 1024, 3584)
        return {'x': _w((lambda *s: _rng.normal(s) * 0.05)(B, S, D)), 'w1': _w((lambda *s: _rng.normal(s) * 0.05)(D, D) * D ** (-0.5)), 'w2': _w((lambda *s: _rng.normal(s) * 0.05)(D, D) * D ** (-0.5)), 'w3': _w((lambda *s: _rng.normal(s) * 0.05)(D, F) * D ** (-0.5)), 'w4': _w((lambda *s: _rng.normal(s) * 0.05)(F, D) * F ** (-0.5))}
    _B_in = _B_setup()
    return {'A_x': _A_in['x'], 'A_wqkv': _A_in['wqkv'], 'A_wo': _A_in['wo'], 'B_x': _B_in['x'], 'B_w1': _B_in['w1'], 'B_w2': _B_in['w2'], 'B_w3': _B_in['w3'], 'B_w4': _B_in['w4'], 'c': _w((lambda *s: _rng.normal(s) * 0.05)(1, 1024)), 'w_mod': _w((lambda *s: _rng.normal(s) * 0.05)(1024, 6 * 1024) * 1024 ** (-0.5))}

def reference(A_x, A_wqkv, A_wo, B_x, B_w1, B_w2, B_w3, B_w4, c, w_mod):

    def _A_ref(x, wqkv, wo):
        B, S, D = x.shape
        H = 32
        Dh = D // H
        W, dil = (8, 2)
        qkv = (lambda x, *d: x.transpose(*d))((x @ wqkv).reshape(B, S, 3, H, Dh), 2, 0, 3, 1, 4)
        q, k, v = (qkv[0], qkv[1], qkv[2])
        scale = Dh ** (-0.5)
        pos = jnp.arange(S)
        off = jnp.arange(W) * dil
        idx = pos[:, None] - off[None, :]
        mask = idx >= 0
        idx_c = jnp.where(mask, idx, 0).reshape(-1)
        kg = k[:, :, idx_c, :].reshape(B, H, S, W, Dh)
        vg = v[:, :, idx_c, :].reshape(B, H, S, W, Dh)
        logits = jnp.einsum('bhsd,bhswd->bhsw', q, kg) * scale
        logits = jnp.where(mask[None, None, :, :], logits, -1000000000.0)
        attn = _softmax(logits, axis=-1)
        o = jnp.einsum('bhsw,bhswd->bhsd', attn, vg)
        return (lambda x, *d: x.transpose(*d))(o, 0, 2, 1, 3).reshape(B, S, D) @ wo

    def _B_ref(x, w1, w2, w3, w4):
        B, S, D = x.shape
        h = _gelu(_layernorm(x, axis=-1) @ w1)
        c = D // 4
        g0 = jnp.pad(h[:, :, 0 * c:1 * c], ((0, 0), (1, 0), (0, 0)))[:, :S, :]
        g1 = jnp.pad(h[:, :, 1 * c:2 * c], ((0, 0), (0, 1), (0, 0)))[:, 1:, :]
        g2 = jnp.pad(h[:, :, 2 * c:3 * c], ((0, 0), (2, 0), (0, 0)))[:, :S, :]
        g3 = jnp.pad(h[:, :, 3 * c:], ((0, 0), (0, 2), (0, 0)))[:, 2:, :]
        hs = jnp.concatenate([g0, g1, g2, g3], axis=-1) @ w2
        x1 = x + hs
        h2 = _gelu(_layernorm(x1, axis=-1) @ w3) @ w4
        return x1 + h2
    x = A_x
    mod = (_silu(c) @ w_mod).reshape(c.shape[0], 6, 1, -1)
    sa, ca, ga, sb, cb, gb = (mod[:, 0].copy(), mod[:, 1].copy(), mod[:, 2].copy(), mod[:, 3].copy(), mod[:, 4].copy(), mod[:, 5].copy())
    h = _layernorm(x, axis=-1) * (1 + ca) + sa
    x = x + ga * _A_ref(h, A_wqkv, A_wo)
    h = _layernorm(x, axis=-1) * (1 + cb) + sb
    x = x + gb * _B_ref(h, B_w1, B_w2, B_w3, B_w4)
    return x
```

```python
import jax
import jax.numpy as jnp
import jax.experimental.pallas as pl
import jax.experimental.pallas.tpu as pltpu

S, D, F, H, DH, W, DIL = 2048, 1024, 3584, 32, 32, 8, 2
T = 256
NT = S // T
FC = 512
HG = 4
PAD = 8
f32, bf16 = jnp.float32, jnp.bfloat16


def _ln(x):
    m = jnp.mean(x, axis=-1, keepdims=True)
    d = x - m
    v = jnp.mean(d * d, axis=-1, keepdims=True)
    return d * jax.lax.rsqrt(v + 1e-5)


def _gelu(x):
    u = x * (0.7978845608028654 + (0.7978845608028654 * 0.044715) * (x * x))
    hx = 0.5 * x
    return hx + hx * jnp.tanh(u)


def _mm(a, b):
    return jnp.dot(a, b, preferred_element_type=f32)


def _body(x_ref, c_ref, wqkv_h, wo_h, w1_h, w2_h, w3_h, w4_h, wm_h, o_ref,
          wqkv, wt, wo, w1, w2, w3, w4, wm, mod, xa, hb, hh, qkv, prev, g_ref, sems):
    i = pl.program_id(0)

    def cp(src, dst, k):
        return pltpu.make_async_copy(src, dst, sems.at[k])

    def cols(h, v, j, k):
        return cp(h.at[:, pl.ds(j * D, D)], v.at[:, pl.ds(j * D, D)], k)

    c_qkv = [cols(wqkv_h, wqkv, j, j) for j in range(3)]
    c_wm = [cols(wm_h, wm, j, 3 + j) for j in range(6)]
    c_wo, c_w1, c_w2 = cp(wo_h, wo, 9), cp(w1_h, w1, 10), cp(w2_h, w2, 11)
    c_w3, c_w4 = cp(w3_h, w3, 12), cp(w4_h, w4, 13)

    def do_mod(j):
        c_wm[j].wait()
        cf = c_ref[...].astype(f32)
        sc = (cf * jax.nn.sigmoid(cf)).astype(bf16)
        mod[j] = _mm(jnp.broadcast_to(sc, (8, D)), wm[:, j * D:(j + 1) * D])

    def stage_a(first):
        off = pl.multiple_of(i * T, T)
        x = x_ref[...].astype(f32)
        h = (_ln(x) * (1.0 + mod[1, 0:1]) + mod[0, 0:1]).astype(bf16)
        qkv[...] = jax.lax.dot_general(wt[...], h, (((1,), (1,)), ((), ())),
                                       preferred_element_type=f32)
        if first:
            c_w2.start()
            c_wm[5].start()
            c_w3.start()
        R = HG * DH
        sub = jax.lax.broadcasted_iota(jnp.int32, (HG, 8, T), 1)
        lane = jax.lax.broadcasted_iota(jnp.int32, (HG, 8, T), 2)
        outs = []
        for g in range(H // HG):
            q = qkv[g * R:(g + 1) * R, :] * (DH ** -0.5)
            ke = jnp.concatenate([prev[g * R:(g + 1) * R, :],
                                  qkv[D + g * R:D + (g + 1) * R, :]], axis=1)
            ve = jnp.concatenate([prev[D + g * R:D + (g + 1) * R, :],
                                  qkv[2 * D + g * R:2 * D + (g + 1) * R, :]], axis=1)

            def sh(e, w):
                return e[:, 128:] if w == 0 else pltpu.roll(e, DIL * w, 1)[:, 128:]

            z = [(q * sh(ke, w)).reshape(HG, 4, 8, T).sum(axis=1) for w in range(W)]
            m4 = (sub & 4) == 0
            z = [jnp.where(m4, z[w], z[w + 4])
                 + pltpu.roll(jnp.where(m4, z[w + 4], z[w]), 4, 1) for w in range(4)]
            for b in (2, 1):
                mb = (sub & b) == 0
                z = [jnp.where(mb, z[w] + pltpu.roll(z[w], 8 - b, 1),
                               z[w + b] + pltpu.roll(z[w + b], b, 1)) for w in range(b)]
            lg = z[0]
            if first:
                lg = jnp.where(lane >= DIL * sub, lg, -1e9)
            e = jnp.exp(lg - jnp.max(lg, axis=1, keepdims=True))
            p = e / jnp.sum(e, axis=1, keepdims=True)
            acc = None
            for w in range(W):
                pw = jnp.broadcast_to(p[:, w:w + 1, :], (HG, 8, T))[:, None]
                t = pw * sh(ve, w).reshape(HG, 4, 8, T)
                acc = t if acc is None else acc + t
            outs.append(acc.reshape(R, T))
        prev[...] = qkv[D:, T - 128:]
        o = jnp.concatenate(outs, axis=0).T.astype(bf16)
        if first:
            do_mod(2)
            c_wo.wait()
        x = x + mod[2, 0:1] * _mm(o, wo[...])
        xa[pl.ds(off, T), :] = x
        if first:
            do_mod(3)
            do_mod(4)
            c_w1.wait()
            c_w4.start()
        h = _ln(x) * (1.0 + mod[4, 0:1]) + mod[3, 0:1]
        hb[pl.ds(off, T), :] = h
        hh[pl.ds(off + PAD, T), :] = _gelu(_mm(_ln(h).astype(bf16), w1[...]))

    def stage_b():
        off = pl.multiple_of((i - 2) * T, T)
        c = D // 4
        hs = jnp.concatenate(
            [hh[pl.ds(off, T + 2 * PAD), j * c:(j + 1) * c][PAD + s:PAD + s + T]
             for j, s in enumerate((-1, 1, -2, 2))], axis=1).astype(bf16)
        x1 = hb[pl.ds(off, T), :] + _mm(hs, w2[...])
        n = _ln(x1).astype(bf16)
        for j in range(F // FC):
            g_ref[:, j * FC:(j + 1) * FC] = _gelu(
                _mm(n, w3[:, j * FC:(j + 1) * FC])).astype(bf16)
        y = x1 + _mm(g_ref[...], w4[...])
        o_ref[...] = (xa[pl.ds(off, T), :] + mod[5, 0:1] * y).astype(o_ref.dtype)

    @pl.when(i == 0)
    def _():
        for j in range(3):
            c_qkv[j].start()
        c_wm[0].start()
        c_wm[1].start()
        prev[...] = jnp.zeros(prev.shape, f32)
        hh[0:PAD, :] = jnp.zeros((PAD, D), f32)
        hh[S + PAD:S + 2 * PAD, :] = jnp.zeros((PAD, D), f32)
        for j in range(3):
            c_qkv[j].wait()
            wt[j * D:(j + 1) * D, :] = wqkv[:, j * D:(j + 1) * D].T
        for d in (c_wm[2], c_wo, c_wm[3], c_wm[4], c_w1):
            d.start()
        do_mod(0)
        do_mod(1)
        stage_a(True)

    @pl.when(i == 1)
    def _():
        stage_a(False)
        c_w2.wait()
        do_mod(5)
        c_w3.wait()
        c_w4.wait()

    @pl.when(jnp.logical_and(i >= 2, i < NT))
    def _():
        stage_a(False)
        stage_b()

    @pl.when(i >= NT)
    def _():
        stage_b()


@jax.jit
def pallas_adaLN_cond__sliding_local_dilated__mixer_s_mlp__prompt_kernel(
        A_x, A_wqkv, A_wo, B_x, B_w1, B_w2, B_w3, B_w4, c, w_mod):
    anyspec = pl.BlockSpec(memory_space=pl.ANY)
    V = pltpu.VMEM
    out = pl.pallas_call(
        _body,
        grid=(NT + 2,),
        in_specs=[pl.BlockSpec((T, D), lambda i: (jnp.minimum(i, NT - 1), 0)),
                  pl.BlockSpec((1, D), lambda i: (0, 0))] + [anyspec] * 7,
        out_specs=pl.BlockSpec((T, D), lambda i: (jnp.maximum(i - 2, 0), 0)),
        out_shape=jax.ShapeDtypeStruct((S, D), A_x.dtype),
        scratch_shapes=[
            V((D, 3 * D), bf16), V((3 * D, D), bf16), V((D, D), bf16), V((D, D), bf16),
            V((D, D), bf16), V((D, F), bf16), V((F, D), bf16), V((D, 6 * D), bf16),
            V((6, 8, D), f32), V((S, D), f32), V((S, D), f32), V((S + 2 * PAD, D), f32),
            V((3 * D, T), f32), V((2 * D, 128), f32), V((T, F), bf16),
            pltpu.SemaphoreType.DMA((14,)),
        ],
        compiler_params=pltpu.CompilerParams(
            dimension_semantics=("arbitrary",), vmem_limit_bytes=110 * 1024 * 1024),
    )(A_x.reshape(S, D), c, A_wqkv, A_wo, B_w1, B_w2, B_w3, B_w4, w_mod)
    return out.reshape(1, S, D)
```

```python
import jax
import jax.numpy as jnp
import jax.experimental.pallas as pl
import jax.experimental.pallas.tpu as pltpu

S, D, F, H, DH, W, DIL = 2048, 1024, 3584, 32, 32, 8, 2
T = 512
NT = S // T
FC = 256
HG = 4
PAD = 8
f32, bf16 = jnp.float32, jnp.bfloat16


def _ln(x):
    m = jnp.mean(x, axis=-1, keepdims=True)
    d = x - m
    v = jnp.mean(d * d, axis=-1, keepdims=True)
    return d * jax.lax.rsqrt(v + 1e-5)


def _gelu(x):
    u = x * (0.7978845608028654 + (0.7978845608028654 * 0.044715) * (x * x))
    hx = 0.5 * x
    return hx + hx * jnp.tanh(u)


def _mm(a, b):
    return jnp.dot(a, b, preferred_element_type=f32)


def _body(x_ref, c_ref, wqkv_h, wo_h, w1_h, w2_h, w3_h, w4_h, wm_h, o_ref,
          wqkv, wt, wo, w1, w2, w3, w4, wm, mod, xa, hb, hh, qkv, prev, ot, nb, up, y, sems):
    i = pl.program_id(0)

    def cp(src, dst, k):
        return pltpu.make_async_copy(src, dst, sems.at[k])

    def cols(h, v, j, k):
        return cp(h.at[:, pl.ds(j * D, D)], v.at[:, pl.ds(j * D, D)], k)

    c_qkv = [cols(wqkv_h, wqkv, j, j) for j in range(3)]
    c_wm = [cols(wm_h, wm, j, 3 + j) for j in range(6)]
    c_wo, c_w1, c_w2 = cp(wo_h, wo, 9), cp(w1_h, w1, 10), cp(w2_h, w2, 11)
    c_w3 = [cp(w3_h.at[:, pl.ds(j * FC, FC)], w3.at[j], 13 + j) for j in range(F // FC)]
    c_w4 = cp(w4_h, w4, 12)

    def do_mod(j):
        c_wm[j].wait()
        cf = c_ref[...].astype(f32)
        sc = (cf * jax.nn.sigmoid(cf)).astype(bf16)
        mod[j] = _mm(jnp.broadcast_to(sc, (8, D)), wm[:, j * D:(j + 1) * D])

    R = HG * DH
    NG = H // HG
    NC = F // FC

    def proj(g, n):
        return jax.lax.dot_general(wt[g], n, (((1,), (1,)), ((), ())),
                                   preferred_element_type=f32)

    def attend(g, r):
        sub = jax.lax.broadcasted_iota(jnp.int32, (HG, 8, T), 1)
        lane = jax.lax.broadcasted_iota(jnp.int32, (HG, 8, T), 2)
        q = r[0:R] * (DH ** -0.5)
        ke = jnp.concatenate([prev[g, 0:R], r[R:2 * R]], axis=1)
        ve = jnp.concatenate([prev[g, R:], r[2 * R:]], axis=1)
        prev[g] = r[R:, T - 128:]

        def sh(e, w):
            return e[:, 128:] if w == 0 else pltpu.roll(e, DIL * w, 1)[:, 128:]

        z = [(q * sh(ke, w)).reshape(HG, 4, 8, T).sum(axis=1) for w in range(W)]
        m4 = (sub & 4) == 0
        z = [jnp.where(m4, z[w], z[w + 4])
             + pltpu.roll(jnp.where(m4, z[w + 4], z[w]), 4, 1) for w in range(4)]
        for b in (2, 1):
            mb = (sub & b) == 0
            z = [jnp.where(mb, z[w] + pltpu.roll(z[w], 8 - b, 1),
                           z[w + b] + pltpu.roll(z[w + b], b, 1)) for w in range(b)]
        lg = jnp.where(lane + i * T >= DIL * sub, z[0], -1e9)
        e = jnp.exp(lg - jnp.max(lg, axis=1, keepdims=True))
        p = e / jnp.sum(e, axis=1, keepdims=True)
        acc = None
        for w in range(W):
            pw = jnp.broadcast_to(p[:, w:w + 1, :], (HG, 8, T))[:, None]
            t = pw * sh(ve, w).reshape(HG, 4, 8, T)
            acc = t if acc is None else acc + t
        ot[g] = acc.reshape(R, T).astype(bf16)

    def stage_a():
        off = pl.multiple_of(i * T, T)
        first = i == 0
        nb[...] = (_ln(x_ref[...].astype(f32)) * (1.0 + mod[1, 0:1])
                   + mod[0, 0:1]).astype(bf16)
        qkv[0] = proj(0, nb[...])

        def grp(g, _):
            attend(g, qkv.at[g % 2])
            qkv[(g + 1) % 2] = proj(g + 1, nb[...])
        jax.lax.fori_loop(0, NG - 1, grp, None)
        attend(NG - 1, qkv.at[(NG - 1) % 2])

        @pl.when(first)
        def _():
            for d in (c_w2, c_wm[5], *c_w3):
                d.start()
            do_mod(2)
            do_mod(3)
            do_mod(4)
            c_wo.wait()
            c_w1.wait()
            c_w4.start()

        o = ot[...].reshape(D, T).T
        x = x_ref[...].astype(f32) + mod[2, 0:1] * _mm(o, wo[...])
        xa[pl.ds(off, T), :] = x
        h = _ln(x) * (1.0 + mod[4, 0:1]) + mod[3, 0:1]
        hb[pl.ds(off, T), :] = h
        hh[pl.ds(off + PAD, T), :] = _gelu(_mm(_ln(h).astype(bf16), w1[...]))

    def stage_b():
        off = pl.multiple_of((i - 2) * T, T)
        c = D // 4
        hs = jnp.concatenate(
            [hh[pl.ds(off, T + 2 * PAD), j * c:(j + 1) * c][PAD + s:PAD + s + T]
             for j, s in enumerate((-1, 1, -2, 2))], axis=1).astype(bf16)
        x1 = hb[pl.ds(off, T), :] + _mm(hs, w2[...])
        y[...] = x1
        nb[...] = _ln(x1).astype(bf16)
        up[0] = _mm(nb[...], w3[0])

        def down(j, k):
            y[...] += _mm(_gelu(up[k]).astype(bf16), w4[j])

        def chunk(j, _):
            down(j, j % 2)
            up[(j + 1) % 2] = _mm(nb[...], w3[j + 1])
        jax.lax.fori_loop(0, NC - 1, chunk, None)
        down(NC - 1, (NC - 1) % 2)
        o_ref[...] = (xa[pl.ds(off, T), :] + mod[5, 0:1] * y[...]).astype(o_ref.dtype)

    @pl.when(i == 0)
    def _():
        for j in range(3):
            c_qkv[j].start()
        c_wm[0].start()
        c_wm[1].start()
        prev[...] = jnp.zeros(prev.shape, f32)
        hh[0:PAD, :] = jnp.zeros((PAD, D), f32)
        hh[S + PAD:S + 2 * PAD, :] = jnp.zeros((PAD, D), f32)
        for j in range(3):
            c_qkv[j].wait()

            def tr(g, _):
                col = pl.multiple_of(j * D + g * R, R)
                wt[g, j * R:(j + 1) * R, :] = wqkv[:, pl.ds(col, R)].T
            jax.lax.fori_loop(0, NG, tr, None)
        for d in (c_wm[2], c_wo, c_wm[3], c_wm[4], c_w1):
            d.start()
        do_mod(0)
        do_mod(1)

    pl.when(i < NT)(stage_a)

    @pl.when(i == 1)
    def _():
        c_w2.wait()
        do_mod(5)
        for d in c_w3:
            d.wait()
        c_w4.wait()

    pl.when(i >= 2)(stage_b)


@jax.jit
def pallas_adaLN_cond__sliding_local_dilated__mixer_s_mlp__prompt_kernel(
        A_x, A_wqkv, A_wo, B_x, B_w1, B_w2, B_w3, B_w4, c, w_mod):
    anyspec = pl.BlockSpec(memory_space=pl.ANY)
    V = pltpu.VMEM
    out = pl.pallas_call(
        _body,
        grid=(NT + 2,),
        in_specs=[pl.BlockSpec((T, D), lambda i: (jnp.minimum(i, NT - 1), 0)),
                  pl.BlockSpec((1, D), lambda i: (0, 0))] + [anyspec] * 7,
        out_specs=pl.BlockSpec((T, D), lambda i: (jnp.maximum(i - 2, 0), 0)),
        out_shape=jax.ShapeDtypeStruct((S, D), A_x.dtype),
        scratch_shapes=[
            V((D, 3 * D), bf16), V((H // HG, 3 * HG * DH, D), bf16), V((D, D), bf16), V((D, D), bf16),
            V((D, D), bf16), V((F // FC, D, FC), bf16), V((F // FC, FC, D), bf16), V((D, 6 * D), bf16),
            V((6, 8, D), f32), V((S, D), f32), V((S, D), f32), V((S + 2 * PAD, D), f32),
            V((2, 3 * HG * DH, T), f32), V((H // HG, 2 * HG * DH, 128), f32),
            V((H // HG, HG * DH, T), bf16), V((T, D), bf16), V((2, T, FC), f32), V((T, D), f32),
            pltpu.SemaphoreType.DMA((13 + F // FC,)),
        ],
        compiler_params=pltpu.CompilerParams(
            dimension_semantics=("arbitrary",), vmem_limit_bytes=110 * 1024 * 1024),
    )(A_x.reshape(S, D), c, A_wqkv, A_wo, B_w1, B_w2, B_w3, B_w4.reshape(F // FC, FC, D), w_mod)
    return out.reshape(1, S, D)
```
